```python
import os as _os
_os.environ.setdefault("JAX_PLATFORMS", "cpu")
import jax
import jax.numpy as jnp

def _softmax(x, axis=-1):
    return jax.nn.softmax(x, axis=axis)
def _gelu(x):
    return jax.nn.gelu(x, approximate=True)
def _silu(x):
    return jax.nn.silu(x)
def _sigmoid(x):
    return jax.nn.sigmoid(x)
def _layernorm(x, axis=-1, eps=1e-5):
    m = jnp.mean(x, axis=axis, keepdims=True)
    v = jnp.var(x, axis=axis, keepdims=True)
    return (x - m) / jnp.sqrt(v + eps)
def _scatter_add(tgt, idx, src, axis=0):
    return tgt.at[idx].add(src)
def _segment_sum(src, seg, n):
    return jax.ops.segment_sum(src, seg, n)
class _Rng:
    def __init__(self, key):
        self._k = key
    def _next(self):
        self._k, sub = jax.random.split(self._k)
        return sub
    def normal(self, shape):
        return jax.random.normal(self._next(), shape, dtype=jnp.bfloat16)
    def randint(self, lo, hi, shape):
        return jax.random.randint(self._next(), shape, lo, hi, dtype=jnp.int32)
    def uniform(self, shape, lo=0.0, hi=1.0):
        return jax.random.uniform(self._next(), shape, jnp.bfloat16, lo, hi)
    def permutation(self, n):
        return jax.random.permutation(self._next(), n)


kernel_name = 'standalone__channel_attn_cbam__vision'

def setup_inputs():
    _rng = _Rng(jax.random.key(int.from_bytes(__import__("os").urandom(4), "little")))
    _w = (lambda a: (lambda t: t.astype(jnp.bfloat16) if jnp.issubdtype(t.dtype, jnp.floating) else t)(jnp.asarray(a)))
    H = W = 384
    C = 192
    r = max(C // 4, 1)
    return {
        "x": _w((lambda *s: _rng.normal(s) * 0.2)(1, H, W, C) + (lambda *s: _rng.normal(s) * 0.2)(1, 1, 1, C) * 2.0),
        "w1": _w((lambda *s: _rng.normal(s) * 0.2)(C, r)),
        "w2": _w((lambda *s: _rng.normal(s) * 0.2)(r, C)),
    }

def reference(x, w1, w2):
    B, H, W, C = x.shape
    xf = x.reshape(B, H * W, C)
    gap = jnp.mean(xf, 1)
    gmp = jnp.amax(xf, 1)
    h_a = gap @ w1
    h_a = h_a * (lambda x, dt: x.astype(dt))(h_a > 0, h_a.dtype)
    h_m = gmp @ w1
    h_m = h_m * (lambda x, dt: x.astype(dt))(h_m > 0, h_m.dtype)
    scale = _sigmoid(h_a @ w2 + h_m @ w2)
    return x * scale[:, None, None, :]
```

```python
import jax
import jax.numpy as jnp
from jax import lax
import jax.experimental.pallas as pl
import jax.experimental.pallas.tpu as pltpu

_ROWS = 8
_WINDOW = 4


def _kernel(x_hbm, w1t_ref, w2_ref, o_hbm, buf, sum_ref, max_ref, sems):
    H, C, W = buf.shape
    n = H // _ROWS

    def read(i):
        rows = pl.ds(i * _ROWS, _ROWS)
        return pltpu.make_async_copy(x_hbm.at[rows], buf.at[rows], sems.at[i % _WINDOW])

    def write(i):
        rows = pl.ds(i * _ROWS, _ROWS)
        return pltpu.make_async_copy(buf.at[rows], o_hbm.at[rows], sems.at[i % _WINDOW])

    for i in range(_WINDOW):
        read(i).start()

    sum_ref[...] = jnp.zeros_like(sum_ref)
    max_ref[...] = jnp.full_like(max_ref, -jnp.inf)

    def pool(i, _):
        read(i).wait()

        @pl.when(i + _WINDOW < n)
        def _():
            read(i + _WINDOW).start()

        for c in range(0, C, 16):
            s = sum_ref[c:c + 16, :]
            m = max_ref[c:c + 16, :]
            for r in range(_ROWS):
                for w in range(0, W, 128):
                    v = buf[i * _ROWS + r, c:c + 16, w:w + 128].astype(jnp.float32)
                    s = s + v
                    m = jnp.maximum(m, v)
            sum_ref[c:c + 16, :] = s
            max_ref[c:c + 16, :] = m

    lax.fori_loop(0, n, pool, None)

    gap = jnp.sum(sum_ref[...], axis=1, keepdims=True) * (1.0 / (H * W))
    gmp = jnp.max(max_ref[...], axis=1, keepdims=True)

    def mlp(g):
        g = jnp.broadcast_to(g, (C, 128)).astype(jnp.bfloat16)
        h = jnp.dot(w1t_ref[...], g, preferred_element_type=jnp.float32)
        h = h.astype(jnp.bfloat16).astype(jnp.float32)
        h = (h * (h > 0).astype(jnp.float32)).astype(jnp.bfloat16)
        y = lax.dot_general(w2_ref[...], h, (((0,), (0,)), ((), ())),
                            preferred_element_type=jnp.float32)
        return y.astype(jnp.bfloat16).astype(jnp.float32)

    z = (mlp(gap) + mlp(gmp)).astype(jnp.bfloat16).astype(jnp.float32)
    scale = jax.nn.sigmoid(z).astype(jnp.bfloat16).astype(jnp.float32)
    sum_ref[...] = scale

    def apply(i, _):
        for c in range(0, C, 16):
            s = sum_ref[c:c + 16, :]
            for r in range(_ROWS):
                for w in range(0, W, 128):
                    v = buf[i * _ROWS + r, c:c + 16, w:w + 128].astype(jnp.float32)
                    buf[i * _ROWS + r, c:c + 16, w:w + 128] = (v * s).astype(jnp.bfloat16)

        @pl.when(i >= _WINDOW)
        def _():
            write(i - _WINDOW).wait()

        write(i).start()

    lax.fori_loop(0, n, apply, None)
    for i in range(n - _WINDOW, n):
        write(i).wait()


@jax.jit
def pallas_standalone__channel_attn_cbam__vision_kernel(
    x: jax.Array,
    w1: jax.Array,
    w2: jax.Array,
):
    B, H, W, C = x.shape
    assert B == 1
    xt = jnp.transpose(x.reshape(H, W, C), (0, 2, 1))
    out = pl.pallas_call(
        _kernel,
        out_shape=jax.ShapeDtypeStruct((H, C, W), x.dtype),
        in_specs=[
            pl.BlockSpec(memory_space=pl.ANY),
            pl.BlockSpec(memory_space=pltpu.VMEM),
            pl.BlockSpec(memory_space=pltpu.VMEM),
        ],
        out_specs=pl.BlockSpec(memory_space=pl.ANY),
        scratch_shapes=[
            pltpu.VMEM((H, C, W), x.dtype),
            pltpu.VMEM((C, 128), jnp.float32),
            pltpu.VMEM((C, 128), jnp.float32),
            pltpu.SemaphoreType.DMA((_WINDOW,)),
        ],
        compiler_params=pltpu.CompilerParams(vmem_limit_bytes=100 * 1024 * 1024),
    )(xt, w1.T, w2)
    return jnp.transpose(out, (0, 2, 1)).reshape(B, H, W, C)
```

```python
import functools

import jax
import jax.numpy as jnp
from jax import lax
import jax.experimental.pallas as pl
import jax.experimental.pallas.tpu as pltpu

_LANES = 128
_TILE = 8
_SLAB = 4096
_PIECE = 64
_PHASES = 9
_PART = 3
_READ_SLABS = 18
_COPY_SLABS = 2
_WRITE_SLABS = 6
_LEAD = 5
_LAG = 4
_RING = 16
_HIGH, _LOW = 0, 1


def _tree(op, vals):
    vals = list(vals)
    while len(vals) > 1:
        vals = [
            op(vals[i], vals[i + 1]) if i + 1 < len(vals) else vals[i]
            for i in range(0, len(vals), 2)
        ]
    return vals[0]


def _rows(index, size):
    start = index * size
    if not isinstance(start, int):
        start = pl.multiple_of(start, size)
    return pl.ds(start, size)


def _cbam_kernel(
    x_hbm, w1t_hbm, w2_hbm, o_hbm,
    buf, w1t_ref, w2_ref, w1_lanes, w2_lanes,
    sum_ref, max_ref, hidden_ref, scale_ref, write_sem,
    *, pixel_tiles,
):
    f32 = jnp.float32
    n_slabs = buf.shape[0]
    n_columns = _SLAB // _PIECE
    n_hidden, n_channels = w2_ref.shape
    n_pixels = n_slabs * _SLAB * _LANES // n_channels
    n_parts = _PHASES // _PART
    part_tiles = n_channels // _TILE // n_parts
    piece_tiles = _PIECE // _TILE
    periods = [g * _PHASES for g in range(n_slabs // _PHASES)]
    n_steps = n_slabs // _READ_SLABS * (n_columns - 1)
    half = _LANES // 2

    def rounded(v):
        return v.astype(buf.dtype).astype(f32)

    def copy(src, dst, slab, slabs, column, sem):
        where = (pl.ds(slab, slabs), _rows(column, _PIECE))
        return pltpu.make_async_copy(src.at[where], dst.at[where], sem)

    read = functools.partial(copy, x_hbm, buf)
    write = functools.partial(copy, buf, o_hbm)

    def cursor(step):
        group, column = divmod(step, n_columns - 1)
        return group * _READ_SLABS, column + 1, (column + 1) % _PHASES

    def advance(cur):
        slab, column, shift = cur
        wrap = column == n_columns - 1
        return (
            jnp.where(wrap, slab + _READ_SLABS, slab),
            jnp.where(wrap, 1, column + 1),
            jnp.where(wrap, 1, jnp.where(shift == _PHASES - 1, 0, shift + 1)),
        )

    def channel_tile(phase, tile):
        return (phase * piece_tiles + tile) // pixel_tiles

    def load_tiles(pieces):
        tiles = {}
        for slab, column, phase in pieces:
            v = buf[slab, _rows(column, _PIECE), :].astype(f32)
            for t in range(piece_tiles):
                tiles.setdefault(channel_tile(phase, t), []).append(
                    v[t * _TILE:(t + 1) * _TILE])
        return tiles

    def pool(pieces):
        for ct, vals in load_tiles(pieces).items():
            sum_ref[ct] = sum_ref[ct] + _tree(jnp.add, vals)
            max_ref[ct] = jnp.maximum(max_ref[ct], _tree(jnp.maximum, vals))

    def pool_step(cur, phases):
        slab, column, shift = cur
        pool([
            (slab + s + jnp.where(p < shift, p - shift + _PHASES, p - shift), column, p)
            for p in phases
            for s in range(0, _READ_SLABS, _PHASES)
        ])

    def rescale(slab, column, scale):
        where = (slab, _rows(column, _PIECE), slice(None))
        buf[where] = (buf[where].astype(f32) * scale).astype(buf.dtype)

    def stream(ring_sems, early_sem, late_sems, weight_sem):
        copies = range(_READ_SLABS // _COPY_SLABS)
        low, high = copies[0::2], copies[1::2]

        def start(k, cur, step):
            read(cur[0] + k * _COPY_SLABS, _COPY_SLABS, cur[1],
                 ring_sems.at[step & (_RING - 1)],
                 ).start(priority=_LOW if k in low else _HIGH)

        def wait(cur, step):
            read(cur[0], _READ_SLABS, cur[1], ring_sems.at[step & (_RING - 1)]).wait()

        early_high = [read(s, _PART, 0, early_sem) for s in periods]
        early_low = [read(s + _PART, _PART, 0, early_sem) for s in periods]
        late_groups = (periods[:-2], periods[-2:])
        late = [
            [read(s + 2 * _PART, _PART, 0, late_sems.at[i]) for s in group]
            for i, group in enumerate(late_groups)
        ]
        weights = [
            pltpu.make_async_copy(w1t_hbm, w1t_ref, weight_sem),
            pltpu.make_async_copy(w2_hbm, w2_ref, weight_sem),
        ]

        for c in early_low:
            c.start(priority=_LOW)
        ahead = [(k, step) for step in range(_LEAD) for k in low]
        for k, step in ahead[:-len(early_high)]:
            start(k, cursor(step), step)
        for c in weights:
            c.start()
        sum_ref[...] = jnp.zeros(sum_ref.shape, f32)
        max_ref[...] = jnp.full(max_ref.shape, -jnp.inf, f32)
        for (k, step), c in zip(ahead[-len(early_high):], early_high):
            start(k, cursor(step), step)
            c.start(priority=_HIGH)
        for i in range(_LAG):
            for k in copies:
                step = i + _LEAD if k in low else i
                start(k, cursor(step), step)

        def steady(i, cursors):
            cur_low, cur_high, cur_pool = cursors
            wait(cur_pool, i - _LAG)
            for k in copies:
                if k in low:
                    start(k, cur_low, i + _LEAD)
                    continue
                start(k, cur_high, i)
                if k // 2 < n_parts:
                    pool_step(cur_pool, range(k // 2 * _PART, (k // 2 + 1) * _PART))
            return advance(cur_low), advance(cur_high), advance(cur_pool)

        end = n_steps - _LEAD
        lax.fori_loop(
            _LAG, end, steady, (cursor(_LAG + _LEAD), cursor(_LAG), cursor(0)))

        pending = late[0] + late[1]
        for step in range(end, n_steps):
            for k in high:
                if pending:
                    pending.pop(0).start(priority=_LOW)
                start(k, cursor(step), step)
        assert not pending

        for c in weights:
            c.wait()
        for src, dst in ((w1t_ref, w1_lanes), (w2_ref, w2_lanes)):
            w = src[...].astype(f32)
            pad = jnp.zeros((half - n_hidden, n_channels), f32)
            dst[...] = jnp.concatenate([w, pad, w, pad], axis=0).T

        for c in early_high + early_low:
            c.wait()

        def pool_early(g, _):
            pool([(g * _PHASES + p, 0, p) for p in range(2 * _PART)])

        lax.fori_loop(0, len(periods), pool_early, None)

        def drain(step, cur):
            wait(cur, step)
            pool_step(cur, range(_PHASES))
            return advance(cur)

        lax.fori_loop(end - _LAG, n_steps, drain, cursor(end - _LAG))

        lane = lax.broadcasted_iota(jnp.int32, (_TILE, _LANES), 1)

        def first_layer(acc, channel_tiles, unpooled):
            for ct in channel_tiles:
                s = _tree(jnp.add, [sum_ref[ct]] + unpooled.get(ct, []))
                m = _tree(jnp.maximum, [max_ref[ct]] + unpooled.get(ct, []))
                gap = jnp.sum(s, axis=1, keepdims=True) * (1.0 / n_pixels)
                gmp = jnp.max(m, axis=1, keepdims=True)
                pooled = rounded(jnp.where(lane < half, gap, gmp))
                acc = acc + pooled * w1_lanes[_rows(ct, _TILE), :]
            return acc

        def landed(i):
            for c in late[i]:
                c.wait()
            return [(s + p, 0, p) for s in late_groups[i]
                    for p in range(2 * _PART, _PHASES)]

        hidden_ref[...] = first_layer(
            jnp.zeros((_TILE, _LANES), f32), range(2 * part_tiles), {})
        pool(landed(0))
        last = load_tiles(landed(1))
        h = first_layer(hidden_ref[...], range(2 * part_tiles, 3 * part_tiles), last)
        h = rounded(jnp.sum(h, axis=0, keepdims=True))
        h = jnp.where((lane & (half - 1)) < n_hidden, h * (h > 0).astype(f32), 0.0)

        def first_column(part, _):
            gates = []
            for i in range(part_tiles):
                w = w2_lanes[_rows(part * part_tiles + i, _TILE), :]
                z = jnp.sum(h * w, axis=1, keepdims=True)
                z = jnp.broadcast_to(z, (_TILE, _LANES))
                gates.append(rounded(jax.nn.sigmoid(rounded(z))))
            scales = [
                jnp.concatenate(
                    [gates[channel_tile(p, t)] for t in range(piece_tiles)], axis=0)
                for p in range(_PART)
            ]
            for s in periods:
                for p in range(_PART):
                    rescale(s + part * _PART + p, 0, scales[p])
                write(s + part * _PART, _PART, 0, write_sem).start()
            for p in range(_PART):
                scale_ref[part * _PART + p] = scales[p]

        lax.fori_loop(0, n_parts, first_column, None)

        def write_group(group, _):
            slab = group * _WRITE_SLABS

            def write_column(column, phase):
                for i in range(_WRITE_SLABS):
                    p = phase + i
                    p = jnp.where(p >= _PHASES, p - _PHASES, p)
                    rescale(slab + i, column, scale_ref[p])
                write(slab, _WRITE_SLABS, column, write_sem).start()
                return jnp.where(phase == _PHASES - 1, 0, phase + 1)

            lax.fori_loop(1, n_columns, write_column, lax.rem(slab + 1, _PHASES))

        lax.fori_loop(0, n_slabs // _WRITE_SLABS, write_group, None)

    sem = pltpu.SemaphoreType.DMA
    pl.run_scoped(stream, sem((_RING,)), sem(()), sem((2,)), sem(()))
    pltpu.make_async_copy(buf, o_hbm, write_sem).wait()


@jax.jit
def pallas_standalone__channel_attn_cbam__vision_kernel(
    x: jax.Array,
    w1: jax.Array,
    w2: jax.Array,
):
    B, H, W, C = x.shape
    pixel_tiles, channel_tiles = W // _LANES, C // _TILE
    assert B == 1 and W % _LANES == 0 and w2.shape[0] < _LANES // 2
    assert C % (_PHASES // _PART * _TILE) == 0
    assert W * C == _PHASES * _PIECE * _LANES
    assert H * W * C % (_READ_SLABS * _SLAB * _LANES) == 0
    shape = (H * W * C // (_SLAB * _LANES), _SLAB, _LANES)

    tiles = x.reshape(H, pixel_tiles, _LANES, channel_tiles, _TILE)
    tiles = tiles.transpose(0, 3, 1, 4, 2).reshape(shape)
    out = pl.pallas_call(
        functools.partial(_cbam_kernel, pixel_tiles=pixel_tiles),
        out_shape=jax.ShapeDtypeStruct(shape, x.dtype),
        in_specs=[pl.BlockSpec(memory_space=pl.ANY)] * 3,
        out_specs=pl.BlockSpec(memory_space=pl.ANY),
        scratch_shapes=[
            pltpu.VMEM(shape, x.dtype),
            pltpu.VMEM(w2.shape, w1.dtype),
            pltpu.VMEM(w2.shape, w2.dtype),
            pltpu.VMEM((C, _LANES), jnp.float32),
            pltpu.VMEM((C, _LANES), jnp.float32),
            pltpu.VMEM((channel_tiles, _TILE, _LANES), jnp.float32),
            pltpu.VMEM((channel_tiles, _TILE, _LANES), jnp.float32),
            pltpu.VMEM((_TILE, _LANES), jnp.float32),
            pltpu.VMEM((_PHASES, _PIECE, _LANES), jnp.float32),
            pltpu.SemaphoreType.DMA(()),
        ],
        compiler_params=pltpu.CompilerParams(vmem_limit_bytes=96 * 1024 * 1024),
    )(tiles, w1.T, w2)
    out = out.reshape(H, channel_tiles, pixel_tiles, _TILE, _LANES)
    return out.transpose(0, 2, 4, 1, 3).reshape(B, H, W, C)
```

```python
import functools

import jax
import jax.numpy as jnp
from jax import lax
import jax.experimental.pallas as pl
import jax.experimental.pallas.tpu as pltpu

_LANES = 128
_TILE = 8
_SLAB = 4096
_PIECE = 64
_PHASES = 9
_PART = 3
_READ_SLABS = 18
_COPY_SLABS = 2
_WRITE_SLABS = 6
_LEAD = 5
_LAG = 4
_RING = 16
_HIGH, _LOW = 0, 1


def _tree(op, vals):
    vals = list(vals)
    while len(vals) > 1:
        vals = [
            op(vals[i], vals[i + 1]) if i + 1 < len(vals) else vals[i]
            for i in range(0, len(vals), 2)
        ]
    return vals[0]


def _rows(index, size):
    start = index * size
    if not isinstance(start, int):
        start = pl.multiple_of(start, size)
    return pl.ds(start, size)


def _cbam_kernel(
    x_hbm, w1t_hbm, w2_hbm, o_hbm,
    buf, w1t_ref, w2_ref, w1_lanes, w2_lanes,
    sum_ref, max_ref, hidden_ref, scale_ref, write_sem,
    *, pixel_tiles,
):
    f32 = jnp.float32
    n_slabs = buf.shape[0]
    n_columns = _SLAB // _PIECE
    n_hidden, n_channels = w2_ref.shape
    n_pixels = n_slabs * _SLAB * _LANES // n_channels
    n_parts = _PHASES // _PART
    part_rows = n_channels // n_parts
    part_tiles = part_rows // _TILE
    piece_tiles = _PIECE // _TILE
    periods = [g * _PHASES for g in range(n_slabs // _PHASES)]
    n_steps = n_slabs // _READ_SLABS * (n_columns - 1)
    half = _LANES // 2

    def rounded(v):
        return v.astype(buf.dtype).astype(f32)

    def copy(src, dst, slab, slabs, column, sem):
        where = (pl.ds(slab, slabs), _rows(column, _PIECE))
        return pltpu.make_async_copy(src.at[where], dst.at[where], sem)

    read = functools.partial(copy, x_hbm, buf)

    def cursor(step):
        group, column = divmod(step, n_columns - 1)
        return group * _READ_SLABS, column + 1, (column + 1) % _PHASES

    def advance(cur):
        slab, column, shift = cur
        wrap = column == n_columns - 1
        return (
            jnp.where(wrap, slab + _READ_SLABS, slab),
            jnp.where(wrap, 1, column + 1),
            jnp.where(wrap, 1, jnp.where(shift == _PHASES - 1, 0, shift + 1)),
        )

    def channel_tile(phase, tile):
        return (phase * piece_tiles + tile) // pixel_tiles

    def pooled(part, periods_of, column, shift):
        tiles = [[] for _ in range(part_tiles)]
        for p in range(_PART):
            offset = part * _PART + p - shift
            if not isinstance(offset, int):
                offset = jnp.where(offset < 0, offset + _PHASES, offset)
            for slab in periods_of:
                v = buf[slab + offset, _rows(column, _PIECE), :].astype(f32)
                for t in range(piece_tiles):
                    tiles[channel_tile(p, t)].append(v[t * _TILE:(t + 1) * _TILE])
        s = jnp.concatenate([_tree(jnp.add, vals) for vals in tiles], axis=0)
        m = jnp.concatenate([_tree(jnp.maximum, vals) for vals in tiles], axis=0)
        return sum_ref[part] + s, jnp.maximum(max_ref[part], m)

    def pool(part, periods_of, column, shift):
        sum_ref[part], max_ref[part] = pooled(part, periods_of, column, shift)

    def pool_step(part, cur):
        slab, column, shift = cur
        pool(part, [slab + s for s in range(0, _READ_SLABS, _PHASES)], column, shift)

    def rescale_and_write(slab, column, scale):
        slabs = scale.shape[0]
        where = (pl.ds(slab, slabs), _rows(column, _PIECE), slice(None))
        buf[where] = (buf[where].astype(f32) * scale).astype(buf.dtype)
        copy(buf, o_hbm, slab, slabs, column, write_sem).start()

    def stream(ring_sems, early_sem, late_sems, weight_sem):
        copies = range(_READ_SLABS // _COPY_SLABS)
        low, high = copies[0::2], copies[1::2]

        def start(k, cur, step):
            read(cur[0] + k * _COPY_SLABS, _COPY_SLABS, cur[1],
                 ring_sems.at[step & (_RING - 1)],
                 ).start(priority=_LOW if k in low else _HIGH)

        def wait(cur, step):
            read(cur[0], _READ_SLABS, cur[1], ring_sems.at[step & (_RING - 1)]).wait()

        early_high = [read(s, _PART, 0, early_sem) for s in periods]
        early_low = [read(s + _PART, _PART, 0, early_sem) for s in periods]
        late_groups = (periods[:-2], periods[-2:])
        late = [
            [read(s + 2 * _PART, _PART, 0, late_sems.at[i]) for s in group]
            for i, group in enumerate(late_groups)
        ]
        weights = [
            pltpu.make_async_copy(w1t_hbm, w1t_ref, weight_sem),
            pltpu.make_async_copy(w2_hbm, w2_ref, weight_sem),
        ]

        for c in early_low:
            c.start(priority=_LOW)
        ahead = [(k, step) for step in range(_LEAD) for k in low]
        for k, step in ahead[:-len(early_high)]:
            start(k, cursor(step), step)
        for c in weights:
            c.start()
        sum_ref[...] = jnp.zeros(sum_ref.shape, f32)
        max_ref[...] = jnp.full(max_ref.shape, -jnp.inf, f32)
        for (k, step), c in zip(ahead[-len(early_high):], early_high):
            start(k, cursor(step), step)
            c.start(priority=_HIGH)
        for i in range(_LAG):
            for k in copies:
                step = i + _LEAD if k in low else i
                start(k, cursor(step), step)

        def steady(i, cursors):
            cur_low, cur_high, cur_pool = cursors
            wait(cur_pool, i - _LAG)
            for k in copies:
                if k in low:
                    start(k, cur_low, i + _LEAD)
                    continue
                start(k, cur_high, i)
                if k // 2 < n_parts:
                    pool_step(k // 2, cur_pool)
            return advance(cur_low), advance(cur_high), advance(cur_pool)

        end = n_steps - _LEAD
        lax.fori_loop(
            _LAG, end, steady, (cursor(_LAG + _LEAD), cursor(_LAG), cursor(0)))

        pending = late[0] + late[1]
        for step in range(end, n_steps):
            for k in high:
                if pending:
                    pending.pop(0).start(priority=_LOW)
                start(k, cursor(step), step)
        assert not pending

        for c in weights:
            c.wait()
        for src, dst in ((w1t_ref, w1_lanes), (w2_ref, w2_lanes)):
            w = src[...].astype(f32)
            pad = jnp.zeros((half - n_hidden, n_channels), f32)
            dst[...] = jnp.concatenate([w, pad, w, pad], axis=0).T

        for c in early_high + early_low:
            c.wait()

        def pool_early(g, _):
            for part in range(n_parts - 1):
                pool(part, [g * _PHASES], 0, 0)

        lax.fori_loop(0, len(periods), pool_early, None)

        def drain(step, cur):
            wait(cur, step)
            for part in range(n_parts):
                pool_step(part, cur)
            return advance(cur)

        lax.fori_loop(end - _LAG, n_steps, drain, cursor(end - _LAG))

        def first_layer(acc, part, s, m):
            gap = jnp.sum(s, axis=1, keepdims=True) * (1.0 / n_pixels)
            gmp = jnp.max(m, axis=1, keepdims=True)
            is_avg = lax.broadcasted_iota(jnp.int32, s.shape, 1) < half
            terms = rounded(jnp.where(is_avg, gap, gmp)) * w1_lanes[_rows(part, part_rows), :]
            for t in range(part_tiles):
                acc = acc + terms[t * _TILE:(t + 1) * _TILE]
            return acc

        h = jnp.zeros((_TILE, _LANES), f32)
        for part in range(n_parts - 1):
            h = first_layer(h, part, sum_ref[part], max_ref[part])
        hidden_ref[...] = h
        for c in late[0]:
            c.wait()
        if late_groups[0]:
            pool(n_parts - 1, late_groups[0], 0, 0)
        for c in late[1]:
            c.wait()
        h = first_layer(
            hidden_ref[...], n_parts - 1, *pooled(n_parts - 1, late_groups[1], 0, 0))
        h = rounded(jnp.sum(h, axis=0, keepdims=True))
        lane = lax.broadcasted_iota(jnp.int32, h.shape, 1)
        h = jnp.where((lane & (half - 1)) < n_hidden, h * (h > 0).astype(f32), 0.0)

        def first_column(part, _):
            z = jnp.sum(h * w2_lanes[_rows(part, part_rows), :], axis=1, keepdims=True)
            z = jnp.broadcast_to(z, (part_rows, _LANES))
            gate = rounded(jax.nn.sigmoid(rounded(z)))
            order = [channel_tile(p, t) for p in range(_PART) for t in range(piece_tiles)]
            scale = jnp.concatenate(
                [gate[ct * _TILE:(ct + 1) * _TILE] for ct in order], axis=0,
            ).reshape(_PART, _PIECE, _LANES)
            for s in periods:
                rescale_and_write(s + part * _PART, 0, scale)
            scale_ref[pl.ds(part * _PART, _PART)] = scale

        lax.fori_loop(0, n_parts, first_column, None)
        scale_ref[pl.ds(_PHASES, _WRITE_SLABS - 1)] = scale_ref[pl.ds(0, _WRITE_SLABS - 1)]

        def write_group(group, _):
            slab = group * _WRITE_SLABS

            def write_column(column, phase):
                rescale_and_write(slab, column, scale_ref[pl.ds(phase, _WRITE_SLABS)])
                return jnp.where(phase == _PHASES - 1, 0, phase + 1)

            lax.fori_loop(1, n_columns, write_column, lax.rem(slab + 1, _PHASES))

        lax.fori_loop(0, n_slabs // _WRITE_SLABS, write_group, None)

    sem = pltpu.SemaphoreType.DMA
    pl.run_scoped(stream, sem((_RING,)), sem(()), sem((2,)), sem(()))
    pltpu.make_async_copy(buf, o_hbm, write_sem).wait()


@jax.jit
def pallas_standalone__channel_attn_cbam__vision_kernel(
    x: jax.Array,
    w1: jax.Array,
    w2: jax.Array,
):
    B, H, W, C = x.shape
    pixel_tiles, channel_tiles = W // _LANES, C // _TILE
    assert B == 1 and W % _LANES == 0 and w2.shape[0] < _LANES // 2
    assert C % (_PHASES // _PART * _TILE) == 0
    assert W * C == _PHASES * _PIECE * _LANES
    assert H * W * C % (_READ_SLABS * _SLAB * _LANES) == 0
    shape = (H * W * C // (_SLAB * _LANES), _SLAB, _LANES)
    stats = (_PHASES // _PART, C * _PART // _PHASES, _LANES)
    scales = (_PHASES + _WRITE_SLABS - 1, _PIECE, _LANES)

    tiles = x.reshape(H, pixel_tiles, _LANES, channel_tiles, _TILE)
    tiles = tiles.transpose(0, 3, 1, 4, 2).reshape(shape)
    out = pl.pallas_call(
        functools.partial(_cbam_kernel, pixel_tiles=pixel_tiles),
        out_shape=jax.ShapeDtypeStruct(shape, x.dtype),
        in_specs=[pl.BlockSpec(memory_space=pl.ANY)] * 3,
        out_specs=pl.BlockSpec(memory_space=pl.ANY),
        scratch_shapes=[
            pltpu.VMEM(shape, x.dtype),
            pltpu.VMEM(w2.shape, w1.dtype),
            pltpu.VMEM(w2.shape, w2.dtype),
            pltpu.VMEM((C, _LANES), jnp.float32),
            pltpu.VMEM((C, _LANES), jnp.float32),
            pltpu.VMEM(stats, jnp.float32),
            pltpu.VMEM(stats, jnp.float32),
            pltpu.VMEM((_TILE, _LANES), jnp.float32),
            pltpu.VMEM(scales, jnp.float32),
            pltpu.SemaphoreType.DMA(()),
        ],
        compiler_params=pltpu.CompilerParams(vmem_limit_bytes=96 * 1024 * 1024),
    )(tiles, w1.T, w2)
    out = out.reshape(H, channel_tiles, pixel_tiles, _TILE, _LANES)
    return out.transpose(0, 2, 4, 1, 3).reshape(B, H, W, C)
```
